```python
import jax
import jax.numpy as jnp

def _softmax(x, axis=-1):
    return jax.nn.softmax(x, axis=axis)

def _gelu(x):
    return jax.nn.gelu(x, approximate=True)

def _silu(x):
    return jax.nn.silu(x)

def _sigmoid(x):
    return jax.nn.sigmoid(x)

def _layernorm(x, axis=-1, eps=1e-05):
    m = jnp.mean(x, axis=axis, keepdims=True)
    v = jnp.var(x, axis=axis, keepdims=True)
    return (x - m) / jnp.sqrt(v + eps)

def _scatter_add(tgt, idx, src, axis=0):
    return tgt.at[idx].add(src)

def _segment_sum(src, seg, n):
    return jax.ops.segment_sum(src, seg, n)

class _Rng:

    def __init__(self, key):
        self._k = key

    def _next(self):
        self._k, sub = jax.random.split(self._k)
        return sub

    def normal(self, shape):
        return jax.random.normal(self._next(), shape, dtype=jnp.bfloat16)

    def randint(self, lo, hi, shape):
        return jax.random.randint(self._next(), shape, lo, hi, dtype=jnp.int32)

    def uniform(self, shape, lo=0.0, hi=1.0):
        return jax.random.uniform(self._next(), shape, jnp.bfloat16, lo, hi)

    def permutation(self, n):
        return jax.random.permutation(self._next(), n)
kernel_name = 'parallel_sum__mha_block__mixer_gmlp__prompt'

def _fwd_setup_inputs():
    _rng = _Rng(jax.random.key(int.from_bytes(__import__("os").urandom(4), "little")))
    _w = lambda a: (lambda t: t.astype(jnp.bfloat16) if jnp.issubdtype(t.dtype, jnp.floating) else t)(jnp.asarray(a))

    def _A_setup():
        B, S, D, H = (1, 2048, 1024, 32)
        return {'x': _w((lambda *s: _rng.normal(s) * 0.05)(B, S, D)), 'wqkv': _w((lambda *s: _rng.normal(s) * 0.05)(D, 3 * D)), 'wo': _w((lambda *s: _rng.normal(s) * 0.05)(D, D))}
    _A_in = _A_setup()

    def _B_setup():
        B, S, D, F = (1, 2048, 1024, 3584)
        Fh = F // 2
        return {'x': _w((lambda *s: _rng.normal(s) * 0.05)(B, S, D)), 'w_in': _w((lambda *s: _rng.normal(s) * 0.05)(D, 2 * Fh)), 'w_sp': _w(0.01 * (lambda *s: _rng.normal(s) * 0.05)(S, S)), 'b_sp': _w(1.0 + 0.01 * (lambda *s: _rng.normal(s) * 0.05)(S)), 'w_out': _w((lambda *s: _rng.normal(s) * 0.05)(Fh, D))}
    _B_in = _B_setup()
    return {'A_x': _A_in['x'], 'A_wqkv': _A_in['wqkv'], 'A_wo': _A_in['wo'], 'B_x': _B_in['x'], 'B_w_in': _B_in['w_in'], 'B_w_sp': _B_in['w_sp'], 'B_b_sp': _B_in['b_sp'], 'B_w_out': _B_in['w_out']}

def _fwd_reference(A_x, A_wqkv, A_wo, B_x, B_w_in, B_w_sp, B_b_sp, B_w_out):

    def _A_ref(x, wqkv, wo):
        B, S, D = x.shape
        H = 32
        Dh = D // H
        qkv = (lambda x, *d: x.transpose(*d))((x @ wqkv).reshape(B, S, 3, H, Dh), 2, 0, 3, 1, 4)
        q, k, v = (qkv[0], qkv[1], qkv[2])
        scores = jnp.einsum('bhqd,bhkd->bhqk', q, k) * Dh ** (-0.5)
        p = _softmax(scores, axis=-1)
        o = jnp.einsum('bhqk,bhkd->bhqd', p, v)
        return (lambda x, *d: x.transpose(*d))(o, 0, 2, 1, 3).reshape(B, S, D) @ wo

    def _B_ref(x, w_in, w_sp, b_sp, w_out):
        B, S, D = x.shape
        F = w_in.shape[-1]
        Fh = F // 2
        z = _gelu(jnp.einsum('bsd,df->bsf', x, w_in))
        z1 = z[..., :Fh].copy()
        z2 = _layernorm(z[..., Fh:], axis=-1)
        g = jnp.einsum('ts,bsf->btf', w_sp, z2) + b_sp[None, :, None]
        return jnp.einsum('bsf,fd->bsd', z1 * g, w_out)
    x = A_x
    xn = _layernorm(x, axis=-1)
    return x + _A_ref(xn, A_wqkv, A_wo) + _B_ref(xn, B_w_in, B_w_sp, B_b_sp, B_w_out)

def setup_inputs():
    _inp = _fwd_setup_inputs()
    _gk = jax.random.fold_in(jax.random.key(int.from_bytes(__import__("os").urandom(4), "little")), 2 ** 31 - 1)
    _shapes = [[1, 2048, 1024]]
    _dtypes = ['bfloat16']
    _gks = jax.random.split(_gk, len(_shapes))
    _gs = [jax.random.normal(k, s, dtype=jnp.dtype(d)) * 0.05 for k, s, d in zip(_gks, _shapes, _dtypes)]
    _inp['grad_out'] = _gs[0]
    return _inp

def reference(A_x, A_wqkv, A_wo, B_w_in, B_w_sp, B_b_sp, B_w_out, B_x, grad_out):
    _const = dict(B_x=B_x)

    def _f(*_d):
        return _fwd_reference(**{'A_x': _d[0], 'A_wqkv': _d[1], 'A_wo': _d[2], 'B_w_in': _d[3], 'B_w_sp': _d[4], 'B_b_sp': _d[5], 'B_w_out': _d[6], **_const})
    _out, _vjp = jax.vjp(_f, A_x, A_wqkv, A_wo, B_w_in, B_w_sp, B_b_sp, B_w_out)
    _grads = _vjp(grad_out)
    _out0 = jnp.asarray(_out)
    return (_out0, *[jnp.asarray(_g) for _g in _grads])
```

```python
import functools
import math

import jax
import jax.numpy as jnp
from jax import lax
import jax.experimental.pallas as pl
import jax.experimental.pallas.tpu as pltpu

S, D, H, DH, F, FH = 2048, 1024, 32, 32, 3584, 1792
BM = 256
NB = S // BM
KC = 128
NKC = S // KC
U = 4
BQ = 512 * U
NQ = S // BQ
NITEM = H * NQ
LAG_K, LAG_O, LAG_S = 2, 2, 4
EPS = 1e-5
SCALE = DH ** -0.5
LOG2E = math.log2(math.e)
LN2 = math.log(2.0)

f32, bf16, u32 = jnp.float32, jnp.bfloat16, jnp.uint32
NN = (((1,), (0,)), ((), ()))
NT = (((1,), (1,)), ((), ()))
TN = (((0,), (0,)), ((), ()))


def _dot(a, b, dn=NN):
    return lax.dot_general(a, b, dn, preferred_element_type=f32)


def _u(x):
    return pltpu.bitcast(x, u32)


def _b(x):
    return pltpu.bitcast(x, bf16)


_cv = lax.convert_element_type


def _r3(x):
    return lax.reshape(x, (KC // 8, 8, 128))


def _rep(x):
    return lax.broadcast_in_dim(x, (KC // 8, 8, 128), (1, 2))


def _ds(i, n):
    if isinstance(i, int):
        return pl.ds(i * n, n)
    return pl.ds(pl.multiple_of(i * n, n), n)


def _gelu_both(h):
    c0 = math.sqrt(2.0 / math.pi)
    c1 = 0.044715
    h2 = h * h
    t = jnp.tanh(h * (c0 + (c0 * c1) * h2))
    a = 0.5 + 0.5 * t
    z = h * a
    gp = a + (0.5 * h) * (1.0 - t * t) * (c0 + (3.0 * c0 * c1) * h2)
    return z, gp


_PATS = (('dp', 'dk', 'dq', 'S', 'dv', 'o'),
         ('dp', 'dk', 'o', 'S', 'dv', 'dq'),
         ('dp', 'dv', 'o', 'S', 'dk', 'dq'),
         ('dp', 'dv', 'dq', 'S', 'dk', 'o'))
_STAGE = {'dp': 'C', 'dv': 'C', 'dk': 'C', 'dq': 'C', 'o': 'B', 'S': 'A'}


def _attn_lists(stages):
    T = NKC * U
    lists = []
    for p in _PATS:
        lk = LAG_K
        lag = {'dp': 0, 'dv': 0, 'dk': lk, 'dq': lk, 'o': LAG_O,
               'S': 0 if 'W' in stages else LAG_S}
        lists.append([('W' if t == 'S' and 'W' in stages else t, r - lag[t])
                      for r in range(T + 8) for t in p
                      if 0 <= r - lag[t] < T
                      and (_STAGE[t] in stages or (t == 'S' and 'W' in stages))])
    return lists


def _zdep(r):
    q = r.shape[0] // 4
    return jnp.concatenate([r[k * q:(k + 1) * q] for k in range(4)], axis=1) * 0.0


def _col(row):
    return jnp.broadcast_to(row, (128, row.shape[1])).T


def _lane_fold(v):
    k = v.shape[1] // 128
    acc = v[:, 0:128]
    for i in range(1, k):
        acc = acc + v[:, i * 128:(i + 1) * 128]
    return acc


def _kernel(x_h, wqkv_h, wo_h, win_h, wsp_h, b_ref, wout_h, dy_h,
            out_h, gx_h, dwqkv_h, dwo_h, dwin_h, dwsp_h, db_ref, dwout_h,
            x_v, dy_v, wqkv_v, wo_v, win_v, wsp_v, wout_v,
            dwo_v, xn_u, oT_u, dqkvT_u, rstd1, dbrow, flag,
            sem_x, sem_dy, sem_w, sem_q, sem_o, sem_s):

    def x_cp(i):
        return pltpu.make_async_copy(x_h.at[_ds(i, BM)], x_v.at[_ds(i, BM)], sem_x.at[i])

    def dy_cp(i):
        return pltpu.make_async_copy(dy_h.at[_ds(i, BM)], dy_v.at[_ds(i, BM)], sem_dy.at[i])

    w_cps = [None] + [pltpu.make_async_copy(h, v, sem_w.at[i]) for i, (h, v) in enumerate(
        [(win_h, win_v), (wsp_h, wsp_v), (wout_h, wout_v)])]

    def wo_cp(c):
        return pltpu.make_async_copy(wo_h.at[_ds(c, BM)], wo_v.at[_ds(c, BM)], sem_w.at[3 + c])

    QW = 512
    NQC = 3 * D // QW

    def wq_cp(c):
        return pltpu.make_async_copy(wqkv_h.at[:, _ds(c, QW)], wqkv_v.at[:, _ds(c, QW)], sem_q.at[c])

    def o_cp(k, src, dst, i, n):
        return pltpu.make_async_copy(src.at[_ds(i, n)], dst.at[_ds(i, n)], sem_o.at[k])

    dwo_cp = pltpu.make_async_copy(dwo_v, dwo_h, sem_o.at[1])

    flag[0] = 1
    dy_cp(0).start()
    for c in range(D // BM):
        wo_cp(c).start()
    x_cp(0).start()
    dy_cp(1).start()
    x_cp(1).start()

    def scope_a(kv_u, qkvT_u, doT_u, sbuf, mbuf, pbuf, smbuf, dk_acc, dv_acc, ds_buf, wacc):
        def p1a(i, carry):
            head = isinstance(i, int)
            dy_cp(i).wait()
            if head:
                dy_cp(2).start()
                x_cp(2).start()
            else:
                x_cp(i).wait()

                @pl.when(i + 2 < NB)
                def _():
                    dy_cp(i + 2).start()
                    x_cp(i + 2).start()

                @pl.when(i >= NB - 3)
                def _():
                    wq_cp(i - (NB - 3)).start()
            rows = _ds(i, BM)
            RP = BM // 4
            stat = {}
            nrm = ((), (), (), (0, 1, 2, 3)) if head else ((), (0, 1), (2, 3), ())
            sts = ((), (), (), (0, 1, 2, 3)) if head else ((0, 1), (2, 3), (), ())
            for c in range(D // BM):
                if head:
                    wo_cp(c).wait()
                    if c == D // BM - 1:
                        x_cp(i).wait()
                doT = _dot(wo_v[c * BM:(c + 1) * BM, :], dy_v[rows, :], NT)
                doT_u[c * BM // 2:(c + 1) * BM // 2, rows] = _u(doT.astype(bf16))
                zd = 0.0 if head else _zdep(doT)
                for kind in ('sn' if head else 'ns'):
                    for p in (nrm if kind == 'n' else sts)[c]:
                        x = x_v[_ds(4 * i + p, RP), :].astype(f32) + zd
                        if kind == 'n':
                            mu, r = stat[p]
                            xn_u[_ds(4 * i + p, RP // 2), :] = _u(((x - mu) * r).astype(bf16))
                        else:
                            mu = jnp.mean(x, axis=-1, keepdims=True)
                            var = jnp.maximum(
                                jnp.mean(x * x, axis=-1, keepdims=True) - mu * mu, 0.0)
                            r = lax.rsqrt(var + EPS)
                            rstd1[_ds(4 * i + p, RP), :] = jnp.broadcast_to(r, (RP, 128))
                            stat[p] = (mu, r)
            return carry
        with jax.named_scope('ph_p1a0'):
            p1a(0, 0)
        with jax.named_scope('ph_p1a'):
            lax.fori_loop(1, NB, p1a, 0)

        def p1b(c, carry):
            wq_cp(c).wait()

            @pl.when(c == 1)
            def _():
                for cp in w_cps[1:]:
                    cp.start()
            is_q = c < D // QW
            sc = jnp.where(is_q, SCALE * LOG2E, 1.0).astype(f32)
            g0 = jnp.where(is_q, 8 + 4 * c, 4 * (c - D // QW))
            w = wqkv_v[:, _ds(c, QW)]
            for i in range(NB):
                rb = (_dot(_b(xn_u[_ds(i, BM // 2), :]), w) * sc).astype(bf16)
                for g in range(QW // 128):
                    kv_u[g0 + g, _ds(i, BM // 2), :] = _u(rb[:, g * 128:(g + 1) * 128])
                qkvT_u[_ds(c, QW // 2), _ds(i, BM)] = _u(rb.T)
            return carry
        for c in range(3, NQC):
            wq_cp(c).start()
        with jax.named_scope('ph_p1b'):
            lax.fori_loop(0, NQC, p1b, 0)

        row_iota = lax.broadcasted_iota(jnp.int32, (64, 128), 0)
        zero_u = jnp.zeros((64, 128), u32)
        KH = KC // 2

        def item(n, stages):
            if 'A' in stages:
                ha, ia = n // NQ, n % NQ
                ga, ja = ha // 4, ha % 4
                mask_a = (row_iota >= ja * 16) & (row_iota < ja * 16 + 16)
            if 'B' in stages:
                hb, ib = (n - 1) // NQ, (n - 1) % NQ
            if 'C' in stages:
                hc, ic = (n - 2) // NQ, (n - 2) % NQ
                gc, jc = hc // 4, hc % 4
                mask_c = (row_iota >= jc * 16) & (row_iota < jc * 16 + 16)
            st = {}
            cnt = {}

            def L(lb):
                return slice(lb * 128, (lb + 1) * 128)

            def Q(i, lb):
                if isinstance(i, int):
                    return pl.ds(i * BQ + lb * 128, 128)
                if NQ == 1:
                    return pl.ds(lb * 128, 128)
                return pl.ds(pl.multiple_of(i * BQ + lb * 128, 128), 128)

            def get(name, lb):
                if (name, lb) in st:
                    return st[name, lb]
                if name == 'qm':
                    v = _b(lax.select(mask_a, qkvT_u[_ds(ga, 64), Q(ia, lb)], zero_u))
                elif name == 'dom':
                    v = _b(lax.select(mask_c, doT_u[_ds(gc, 64), Q(ic, lb)], zero_u))
                elif name == 'mb':
                    v = _rep(mbuf[:, L(lb)])
                elif name == 'delta':
                    v = _rep(smbuf[0:8, L(lb)])
                elif name == 'linv':
                    v = lax.concatenate([smbuf[8:16, L(lb)]] * 4, 0)
                elif name == 'qs':
                    v = (_b(qkvT_u[_ds(hc, 16), Q(ic, lb)]).astype(f32)
                         * (get('linv', lb) * LN2)).astype(bf16)
                elif name == 'dos':
                    v = (_b(doT_u[_ds(hc, 16), Q(ic, lb)]).astype(f32) * get('linv', lb)).astype(bf16)
                st[name, lb] = v
                return v

            def accum(key, c, r, f=lax.add):
                st[key] = r if c == 0 else f(st[key], r)

            def op(t, tt, j):
                u, c = tt // NKC, tt % NKC
                lb = u * 4 + j
                ks = _ds(c, KC)
                hs = _ds(c, KH)
                dsl = (_ds(tt % 4, KH), L(j))
                if t == 'W':
                    jb = (0 if 'B' in stages else 2) + lb // 8
                    r = _dot(_b(oT_u[_ds(jb, BM // 2), ks]), dy_v[ks, L(lb % 8)])
                    if c > 0:
                        r = lax.add(r, wacc[j])
                    if c < NKC - 1:
                        wacc[j] = r
                    else:
                        dwo_v[_ds(jb, BM), L(lb % 8)] = r.astype(bf16)
                elif t == 'S':
                    sc = _dot(_b(kv_u[ga, hs, :]), get('qm', lb))
                    sbuf[ks, L(lb)] = sc
                    accum(('m', lb), c, lax.reduce_max(_r3(sc), (0,)), lax.max)
                    if c == NKC - 1:
                        mbuf[:, L(lb)] = jnp.broadcast_to(
                            jnp.max(st['m', lb], axis=0, keepdims=True), (8, 128))
                elif t == 'dp':
                    dp = _dot(_b(kv_u[8 + gc, hs, :]), get('dom', lb))
                    pc = _r3(_cv(_b(pbuf[hs, L(lb)]), f32))
                    ds = lax.mul(pc, lax.sub(_r3(dp), get('delta', lb)))
                    ds_buf[dsl] = _u(_cv(lax.reshape(ds, (KC, 128)), bf16))
                elif t == 'exp':
                    p = lax.exp2(lax.sub(_r3(sbuf[ks, L(lb)]), get('mb', lb)))
                    accum(('l', lb), c, lax.reduce_sum(p, (0,)))
                    p = lax.reshape(p, (KC, 128))
                    pl8 = lax.slice(p, (KC - 8, 0), (KC, 128))
                    pl8 = lax.min(pl8, lax.add(pl8, st['l', lb]))
                    p = lax.concatenate([lax.slice(p, (0, 0), (KC - 8, 128)), pl8], 0)
                    pbuf[hs, L(lb)] = _u(_cv(p, bf16))
                elif t == 'o':
                    accum(('o', lb), c,
                          _dot(_b(qkvT_u[_ds(2 * H + hb, 16), ks]), _b(pbuf[hs, L(lb)])))
                    if c == NKC - 1:
                        li = 1.0 / jnp.sum(st['l', lb], axis=0, keepdims=True)
                        o = st['o', lb] * li
                        oT_u[_ds(hb, 16), Q(ib, lb)] = _u(o.astype(bf16))
                        dO = _b(doT_u[_ds(hb, 16), Q(ib, lb)]).astype(f32)
                        dl = jnp.sum(o * dO, axis=0, keepdims=True)
                        smbuf[:, L(lb)] = jnp.concatenate(
                            [jnp.broadcast_to(dl, (8, 128)), jnp.broadcast_to(li, (8, 128))], axis=0)
                elif t == 'dq':
                    accum(('dq', lb), c, _dot(_b(qkvT_u[_ds(H + hc, 16), ks]), _b(ds_buf[dsl])))
                    if c == NKC - 1:
                        dqkvT_u[_ds(hc, 16), Q(ic, lb)] = _u(
                            (st['dq', lb] * (get('linv', lb) * SCALE)).astype(bf16))
                else:
                    if t == 'dk':
                        acc, off = dk_acc, H
                        r = _dot(get('qs', lb), _b(ds_buf[dsl]), NT)
                    else:
                        acc, off = dv_acc, 2 * H
                        r = _dot(get('dos', lb), _b(pbuf[hs, L(lb)]), NT)
                    k = cnt.get((t, tt), 0)
                    cnt[t, tt] = k + 1
                    accum((t, tt), k, r)
                    if k == 3:
                        tot = st[t, tt]
                        if u > 0:
                            tot = lax.add(acc[:, ks], tot)
                        if u < U - 1:
                            acc[:, ks] = tot
                        else:
                            dqkvT_u[_ds(off + hc, 16), ks] = _u(_cv(tot, bf16))

            lists = _attn_lists(stages)
            cdone = {}
            for k in range(len(lists[0])):
                for j in range(4):
                    t, tt = lists[j][k]
                    if t == 'o' and 'C' not in stages:
                        if tt == 0:
                            op('exp', 0, j)
                        if tt + 1 < NKC * U:
                            op('exp', tt + 1, j)
                    op(t, tt, j)
                    if t in ('dp', 'dv') and 'B' in stages:
                        cdone[tt, j] = cdone.get((tt, j), 0) + 1
                        if cdone[tt, j] == 2:
                            op('exp', tt, j)

        def block(n, stages):
            with jax.named_scope('ph_a' + stages):
                pl.when(flag[0] == 1)(functools.partial(item, n, stages))

        def abody(n, carry):
            item(n, 'ABC')
            return carry
        block(0, 'A')
        block(1, 'AB')
        with jax.named_scope('ph_aABC'):
            lax.fori_loop(2, NITEM, abody, 0)
        block(NITEM, 'BCW')
        block(NITEM + 1, 'CW')
        dwo_cp.start()

    pl.run_scoped(
        scope_a,
        pltpu.VMEM((16, S // 2, 128), u32),
        pltpu.VMEM((3 * D // 2, S), u32),
        pltpu.VMEM((D // 2, S), u32),
        pltpu.VMEM((S, BQ), f32), pltpu.VMEM((8, BQ), f32),
        pltpu.VMEM((S // 2, BQ), u32), pltpu.VMEM((16, BQ), f32),
        pltpu.VMEM((32, S), f32), pltpu.VMEM((32, S), f32),
        pltpu.VMEM((4 * KC // 2, 512), u32),
        pltpu.VMEM((4, BM, 128), f32),
    )

    CW = 256
    NCH = FH // CW

    def scope_b(z1_u, z2n_u, gp_u, dg_u, tmp, wT_u, rstd2, stage, s12, uT_u):
        w_cps[1].wait()

        def b0(i, carry):
            rows = _ds(i, BM)
            hrows = _ds(i, BM // 2)
            xn = _b(xn_u[hrows, :])
            for c in range(NCH):
                cs = slice(c * CW, (c + 1) * CW)
                cs2 = slice(FH + c * CW, FH + (c + 1) * CW)
                h = _dot(xn, win_v[:, cs2])
                if c > 0:
                    h = h + jnp.concatenate([ssum, vsum], axis=1) * 0.0
                z, gp = _gelu_both(h)
                tmp[:, cs] = z
                gp_u[hrows, cs2] = _u(gp.astype(bf16))
                ssum = _lane_fold(z) if c == 0 else ssum + _lane_fold(z)
                vsum = _lane_fold(z * z) if c == 0 else vsum + _lane_fold(z * z)
            mu = jnp.sum(ssum, axis=-1, keepdims=True) * (1.0 / FH)
            var = jnp.maximum(jnp.sum(vsum, axis=-1, keepdims=True) * (1.0 / FH) - mu * mu, 0.0)
            r = jnp.broadcast_to(lax.rsqrt(var + EPS), (BM, 128))
            rstd2[rows, :] = r
            r = jnp.tile(r, (1, CW // 128))
            mu = jnp.tile(jnp.broadcast_to(mu, (BM, 128)), (1, CW // 128))
            for c in range(NCH):
                cs = slice(c * CW, (c + 1) * CW)
                h = _dot(xn, win_v[:, cs])
                z, gp = _gelu_both(h)
                z1_u[hrows, cs] = _u(z.astype(bf16))
                gp_u[hrows, cs] = _u(gp.astype(bf16))
                for cc in ((), (0,), (1, 2), (3,), (4,), (5,), (6,))[c]:
                    ccs = slice(cc * CW, (cc + 1) * CW)
                    z2n_u[hrows, ccs] = _u(((tmp[:, ccs] - (mu + h * 0.0)) * r).astype(bf16))
            return carry
        with jax.named_scope('ph_b0'):
            lax.fori_loop(0, NB, b0, 0)

        w_cps[2].wait()
        w_cps[3].wait()
        dbrow[...] = b_ref[...].astype(f32).reshape(1, S)

        def b1(i, carry):
            rows = _ds(i, BM)
            hrows = _ds(i, BM // 2)
            bcol = jnp.tile(_col(dbrow[:, rows]), (1, CW // 128))
            wsp_t = wsp_v[rows, :]
            dy_t = dy_v[rows, :]
            dbacc = jnp.zeros((BM, 128), f32)
            for c in range(NCH):
                cs = slice(c * CW, (c + 1) * CW)
                g = _dot(wsp_t, _b(z2n_u[:, cs])) + bcol
                du = _dot(dy_t, wout_v[cs, :], NT)
                z1 = _b(z1_u[hrows, cs]).astype(f32)
                gp1 = _b(gp_u[hrows, cs]).astype(f32)
                dg = du * z1
                dbacc = dbacc + _lane_fold(dg)
                ub = (z1 * g).astype(bf16)
                z1_u[hrows, cs] = _u(ub)
                uT_u[c * CW // 2:(c + 1) * CW // 2, rows] = _u(ub.T)
                dg_u[hrows, cs] = _u(dg.astype(bf16))
                gp_u[hrows, cs] = _u((du * g * gp1).astype(bf16))
            o = _dot(_b(oT_u[:, rows]), wo_v[...], TN)
            o = o + _dot(_b(z1_u[hrows, :]), wout_v[...])
            x_v[rows, :] = (x_v[rows, :].astype(f32) + o).astype(bf16)
            o_cp(0, x_v, out_h, i, BM).start()
            dbrow[:, rows] = jnp.sum(dbacc.T, axis=0, keepdims=True)
            return carry
        with jax.named_scope('ph_b1'):
            lax.fori_loop(0, NB, b1, 0)
        db_ref[...] = dbrow[...].reshape(S).astype(bf16)

        SW = 512
        FB = FH // NB

        def dwsp_cp(i):
            return pltpu.make_async_copy(stage.at[i % 2], dwsp_h.at[_ds(i, BM)], sem_s.at[i % 2])

        def w2a(i, carry):
            rows = _ds(i, BM)

            @pl.when(i >= 2)
            def _():
                dwsp_cp(i - 2).wait()
            dbcol = jnp.tile(_col(dbrow[:, rows]), (1, SW // 128))
            dg_t = _b(dg_u[_ds(i, BM // 2), :])
            for c in range(S // SW):
                cs = slice(c * SW, (c + 1) * SW)
                d = _dot(dg_t, _b(z2n_u[c * SW // 2:(c + 1) * SW // 2, :]), NT)
                w = wsp_v[rows, cs].astype(f32)
                wb = (w * dbcol).reshape(BM // 16, 2, 8, SW)
                wd = (w * d).reshape(BM // 16, 2, 8, SW)
                d4 = d.reshape(BM // 16, 2, 8, SW)
                outs = []
                for g in range(BM // 16):
                    if g == 0:
                        outs.append(d4[g, 0] if c == 0 else d4[g, 0] + (p1 + p2) * 0.0)
                        p1 = jnp.where(i == 0, 0.0, s12[0:8, cs])
                        p2 = jnp.where(i == 0, 0.0, s12[8:16, cs])
                    else:
                        outs.append(d4[g, 0] + (p1 + p2) * 0.0)
                    outs.append(d4[g, 1])
                    p1 = p1 + (wb[g, 0] + wb[g, 1])
                    p2 = p2 + (wd[g, 0] + wd[g, 1])
                stage[i % 2, :, cs] = jnp.concatenate(outs, axis=0).astype(bf16)
                s12[0:8, cs] = p1
                s12[8:16, cs] = p2
            wT_u[...] = _u(wsp_v[:, 0:BM].T)
            wout_v[_ds(i, FB), :] = _dot(_b(uT_u[_ds(i, FB // 2), :]), dy_v[...]).astype(bf16)
            dwsp_cp(i).start()
            o_cp(2, wout_v, dwout_h, i, FB).start()
            return carry
        with jax.named_scope('ph_w2a'):
            lax.fori_loop(0, NB, w2a, 0)

        def ln1_a(blk, p, n, dep):
            k = blk * (BM // n) + p
            dxn = tmp[_ds(p, n), 0:D]
            if dep is not None:
                dxn = dxn + dep
            xn = _b(xn_u[_ds(k, n // 2), :]).astype(f32)
            a1 = jnp.mean(dxn, axis=-1, keepdims=True)
            a2 = jnp.mean(dxn * xn, axis=-1, keepdims=True)
            return a1, a2

        def ln1_b(blk, p, n, a12, valid, dep):
            k = blk * (BM // n) + p
            rows = _ds(k, n)
            dxn = tmp[_ds(p, n), 0:D]
            if dep is not None:
                dxn = dxn + dep
            xn = _b(xn_u[_ds(k, n // 2), :]).astype(f32)
            r1 = jnp.tile(rstd1[rows, :], (1, D // 128))
            upd = r1 * (dxn - a12[0] - xn * a12[1])
            if valid is not None:
                upd = jnp.where(valid, upd, 0.0)
            dy_v[rows, :] = (dy_v[rows, :].astype(f32) + upd).astype(bf16)

        def b2(i, carry):
            rows = _ds(i, BM)
            hrows = _ds(i, BM // 2)
            ip = jnp.maximum(i - 1, 0)
            r2 = rstd2[rows, :]
            s12r = s12[:, rows]
            c1 = _col(jnp.sum(s12r[0:8], axis=0, keepdims=True)) * (r2 * (1.0 / FH))
            c2 = _col(jnp.sum(s12r[8:16], axis=0, keepdims=True)) * (r2 * (1.0 / FH))
            r2, c1, c2 = (jnp.tile(v, (1, CW // 128)) for v in (r2, c1, c2))
            for c in range(NCH):
                cs = slice(c * CW, (c + 1) * CW)
                cs2 = slice(FH + c * CW, FH + (c + 1) * CW)
                dz = _dot(_b(wT_u[...]), _b(dg_u[:, cs]))
                z2n = _b(z2n_u[hrows, cs]).astype(f32)
                gp2 = _b(gp_u[hrows, cs2]).astype(f32)
                gp_u[hrows, cs2] = _u((gp2 * (r2 * dz - c1 - z2n * c2)).astype(bf16))
                if 1 <= c <= 4:
                    ln1_b(ip, c - 1, BM // 4, a12, i > 0, _zdep(dz))
                if c < 4:
                    a12 = ln1_a(ip, c, BM // 4, _zdep(dz))
            dxa = _dot(wqkv_v[...], _b(dqkvT_u[:, rows]))
            wT_u[...] = _u(wsp_v[:, _ds(jnp.minimum(i + 1, NB - 1), BM)].T)
            tmp[:, 0:D] = dxa.T + _dot(_b(gp_u[hrows, :]), win_v[...], NT)

            @pl.when(i > 0)
            def _():
                o_cp(3, dy_v, gx_h, ip, BM).start()
            return carry
        with jax.named_scope('ph_b2'):
            lax.fori_loop(0, NB, b2, 0)

        BW = 128

        def w2b(i, carry):
            rows = _ds(i, BW)
            wT_u[0:BW // 2, :] = _u(_b(xn_u[:, rows]).T)
            xT = _b(wT_u[0:BW // 2, :])
            GP = BM // (D // BW)
            for c in range(3):
                r = _dot(xT, _b(dqkvT_u[c * D // 2:(c + 1) * D // 2, :]), NT)
                wqkv_v[rows, c * D:(c + 1) * D] = r.astype(bf16)
                if c == 0:
                    a12 = ln1_a(NB - 1, i, GP, r[0:GP] * 0.0)
                if c == 1:
                    ln1_b(NB - 1, i, GP, a12, None, r[0:GP] * 0.0)
            o_cp(5, wqkv_v, dwqkv_h, i, BW).start()
            o_cp(4, dy_v, gx_h, (NB - 1) * (BM // GP) + i, GP).start()
            win_v[rows, :] = _dot(xT, _b(gp_u[...])).astype(bf16)
            o_cp(6, win_v, dwin_h, i, BW).start()
            return carry
        with jax.named_scope('ph_w2b'):
            lax.fori_loop(0, D // BW, w2b, 0)

        with jax.named_scope('ph_final'):
            for i in range(NB):
                o_cp(0, x_v, out_h, i, BM).wait()
                if i < NB - 1:
                    o_cp(3, dy_v, gx_h, i, BM).wait()
            dwsp_cp(NB - 2).wait()
            dwsp_cp(NB - 1).wait()
            dwo_cp.wait()
            for i in range(NB):
                o_cp(2, wout_v, dwout_h, i, FB).wait()
            for i in range(D // BW):
                o_cp(5, wqkv_v, dwqkv_h, i, BW).wait()
                o_cp(4, dy_v, gx_h, (NB - 1) * (D // BW) + i, BM // (D // BW)).wait()
                o_cp(6, win_v, dwin_h, i, BW).wait()

    pl.run_scoped(
        scope_b,
        pltpu.VMEM((S // 2, FH), u32),
        pltpu.VMEM((S // 2, FH), u32),
        pltpu.VMEM((S // 2, F), u32),
        pltpu.VMEM((S // 2, FH), u32),
        pltpu.VMEM((BM, FH), f32),
        pltpu.VMEM((BM // 2, S), u32),
        pltpu.VMEM((S, 128), f32),
        pltpu.VMEM((2, BM, S), bf16),
        pltpu.VMEM((16, S), f32),
        pltpu.VMEM((FH // 2, S), u32),
    )


@jax.jit
def pallas_parallel_sum__mha_block__mixer_gmlp__prompt_kernel(
    A_x: jax.Array,
    A_wqkv: jax.Array,
    A_wo: jax.Array,
    B_x: jax.Array,
    B_w_in: jax.Array,
    B_w_sp: jax.Array,
    B_b_sp: jax.Array,
    B_w_out: jax.Array,
    grad_out: jax.Array,
):
    del B_x
    x = A_x.reshape(S, D)
    dy = grad_out.reshape(S, D)
    hbm = pl.BlockSpec(memory_space=pl.ANY)
    vmem = pl.BlockSpec(memory_space=pltpu.VMEM)
    out_shape = (
        jax.ShapeDtypeStruct((S, D), bf16),
        jax.ShapeDtypeStruct((S, D), bf16),
        jax.ShapeDtypeStruct((D, 3 * D), bf16),
        jax.ShapeDtypeStruct((D, D), bf16),
        jax.ShapeDtypeStruct((D, F), bf16),
        jax.ShapeDtypeStruct((S, S), bf16),
        jax.ShapeDtypeStruct((S,), bf16),
        jax.ShapeDtypeStruct((FH, D), bf16),
    )
    outs = pl.pallas_call(
        _kernel,
        out_shape=out_shape,
        in_specs=[hbm, hbm, hbm, hbm, hbm, vmem, hbm, hbm],
        out_specs=(hbm, hbm, hbm, hbm, hbm, hbm, vmem, hbm),
        scratch_shapes=[
            pltpu.VMEM((S, D), bf16), pltpu.VMEM((S, D), bf16),
            pltpu.VMEM((D, 3 * D), bf16), pltpu.VMEM((D, D), bf16),
            pltpu.VMEM((D, F), bf16), pltpu.VMEM((S, S), bf16), pltpu.VMEM((FH, D), bf16),
            pltpu.VMEM((D, D), bf16),
            pltpu.VMEM((S // 2, D), u32), pltpu.VMEM((D // 2, S), u32),
            pltpu.VMEM((3 * D // 2, S), u32), pltpu.VMEM((S, 128), f32),
            pltpu.VMEM((1, S), f32), pltpu.SMEM((1,), jnp.int32),
            pltpu.SemaphoreType.DMA((NB,)), pltpu.SemaphoreType.DMA((NB,)),
            pltpu.SemaphoreType.DMA((7,)), pltpu.SemaphoreType.DMA((6,)), pltpu.SemaphoreType.DMA((7,)),
            pltpu.SemaphoreType.DMA((2,)),
        ],
        compiler_params=pltpu.CompilerParams(vmem_limit_bytes=120 * 1024 * 1024),
        name="fused_fwd_bwd",
    )(x, A_wqkv, A_wo, B_w_in, B_w_sp, B_b_sp, B_w_out, dy)
    out, gx, dwqkv, dwo, dwin, dwsp, db, dwout = outs
    return (out.reshape(1, S, D), gx.reshape(1, S, D), dwqkv, dwo, dwin, dwsp, db, dwout)
```
